```python
import os as _os
_os.environ.setdefault("JAX_PLATFORMS", "cpu")
import jax
import jax.numpy as jnp

def _softmax(x, axis=-1):
    return jax.nn.softmax(x, axis=axis)
def _gelu(x):
    return jax.nn.gelu(x, approximate=True)
def _silu(x):
    return jax.nn.silu(x)
def _sigmoid(x):
    return jax.nn.sigmoid(x)
def _layernorm(x, axis=-1, eps=1e-5):
    m = jnp.mean(x, axis=axis, keepdims=True)
    v = jnp.var(x, axis=axis, keepdims=True)
    return (x - m) / jnp.sqrt(v + eps)
def _scatter_add(tgt, idx, src, axis=0):
    return tgt.at[idx].add(src)
def _segment_sum(src, seg, n):
    return jax.ops.segment_sum(src, seg, n)
class _Rng:
    def __init__(self, key):
        self._k = key
    def _next(self):
        self._k, sub = jax.random.split(self._k)
        return sub
    def normal(self, shape):
        return jax.random.normal(self._next(), shape, dtype=jnp.bfloat16)
    def randint(self, lo, hi, shape):
        return jax.random.randint(self._next(), shape, lo, hi, dtype=jnp.int32)
    def uniform(self, shape, lo=0.0, hi=1.0):
        return jax.random.uniform(self._next(), shape, jnp.bfloat16, lo, hi)
    def permutation(self, n):
        return jax.random.permutation(self._next(), n)


kernel_name = 'concat_heads__gqa_block_cached__gqa_block_cached__near_ridge'

def setup_inputs():
    _rng = _Rng(jax.random.key(int.from_bytes(__import__("os").urandom(4), "little")))
    _w = (lambda a: (lambda t: t.astype(jnp.bfloat16) if jnp.issubdtype(t.dtype, jnp.floating) else t)(jnp.asarray(a)))
    def _A_setup():
        B, Sq, D = 8, 240, 640
        Hq, Hkv, Sk, Dh = 32, 32, 1024, 192
        assert Hq % Hkv == 0, (Hq, Hkv)
        return {
            "x": _w((lambda *s: _rng.normal(s) * 0.8)(B, Sq, D)),
            "k_cache": _w((lambda *s: _rng.normal(s) * 0.8)(B, Hkv, Sk, Dh)),
            "v_cache": _w((lambda *s: _rng.normal(s) * 0.05)(B, Hkv, Sk, Dh)),
            "wq": _w((lambda *s: _rng.normal(s) * 0.8)(D, Hq * Dh) * (D ** -0.5)),
            "wo": _w((lambda *s: _rng.normal(s) * 0.05)(Hq * Dh, D) * ((Hq * Dh) ** -0.5)),
        }
    _A_in = _A_setup()

    def _B_setup():
        B, Sq, D = 8, 240, 640
        Hq, Hkv, Sk, Dh = 32, 32, 1024, 192
        assert Hq % Hkv == 0, (Hq, Hkv)
        return {
            "x": _w((lambda *s: _rng.normal(s) * 0.8)(B, Sq, D)),
            "k_cache": _w((lambda *s: _rng.normal(s) * 0.8)(B, Hkv, Sk, Dh)),
            "v_cache": _w((lambda *s: _rng.normal(s) * 0.05)(B, Hkv, Sk, Dh)),
            "wq": _w((lambda *s: _rng.normal(s) * 0.8)(D, Hq * Dh) * (D ** -0.5)),
            "wo": _w((lambda *s: _rng.normal(s) * 0.05)(Hq * Dh, D) * ((Hq * Dh) ** -0.5)),
        }
    _B_in = _B_setup()

    return {
        "A_x": _A_in["x"],
        "A_k_cache": _A_in["k_cache"],
        "A_v_cache": _A_in["v_cache"],
        "A_wq": _A_in["wq"],
        "A_wo": _A_in["wo"],
        "B_x": _B_in["x"],
        "B_k_cache": _B_in["k_cache"],
        "B_v_cache": _B_in["v_cache"],
        "B_wq": _B_in["wq"],
        "B_wo": _B_in["wo"],
    }

def reference(A_x, A_k_cache, A_v_cache, A_wq, A_wo, B_x, B_k_cache, B_v_cache, B_wq, B_wo):
    def _A_ref(x, k_cache, v_cache, wq, wo):
        B, Sq, D = x.shape
        Hq, Dh = 32, 192
        Hkv = k_cache.shape[1]
        rep = Hq // Hkv
        q = (lambda x, *d: x.transpose(*d))((x @ wq).reshape(B, Sq, Hq, Dh), 0, 2, 1, 3)
        k = jnp.repeat(k_cache, rep, axis=1)
        v = jnp.repeat(v_cache, rep, axis=1)
        scores = jnp.einsum("bhqd,bhkd->bhqk", q, k) * (Dh ** -0.5)
        p = _softmax(scores, axis=-1)
        o = jnp.einsum("bhqk,bhkd->bhqd", p, v)
        return (lambda x, *d: x.transpose(*d))(o, 0, 2, 1, 3).reshape(B, Sq, Hq * Dh) @ wo

    def _B_ref(x, k_cache, v_cache, wq, wo):
        B, Sq, D = x.shape
        Hq, Dh = 32, 192
        Hkv = k_cache.shape[1]
        rep = Hq // Hkv
        q = (lambda x, *d: x.transpose(*d))((x @ wq).reshape(B, Sq, Hq, Dh), 0, 2, 1, 3)
        k = jnp.repeat(k_cache, rep, axis=1)
        v = jnp.repeat(v_cache, rep, axis=1)
        scores = jnp.einsum("bhqd,bhkd->bhqk", q, k) * (Dh ** -0.5)
        p = _softmax(scores, axis=-1)
        o = jnp.einsum("bhqk,bhkd->bhqd", p, v)
        return (lambda x, *d: x.transpose(*d))(o, 0, 2, 1, 3).reshape(B, Sq, Hq * Dh) @ wo

    a = _A_ref(A_x, A_k_cache, A_v_cache, A_wq, A_wo)
    b = _B_ref(B_x, B_k_cache, B_v_cache, B_wq, B_wo)
    return jnp.concatenate([a, b], axis=-1)
```

```python
import jax
import jax.numpy as jnp
import numpy as np
from jax import lax
import jax.experimental.pallas as pl
import jax.experimental.pallas.tpu as pltpu

B, SQ, D = 8, 240, 640
H, SK, DH = 32, 1024, 192
NPAIR = H // 2
NJ = NPAIR * B
PW = 2 * DH
SCALE = DH ** -0.5
LOG2E = float(np.log2(np.e))
F32 = jnp.float32
BF16 = jnp.bfloat16
U32 = jnp.uint32
NT = (((1,), (1,)), ((), ()))

R = 2
RC = 16
CW = 512
SP = 256
PO = SQ
MO = PO + SP // 2
XR_ = MO + SP
NZ = 3


def _kernel(xa_hbm, xb_hbm, ka_hbm, va_hbm, kb_hbm, vb_hbm, wqa_hbm, woa_hbm, wqb_hbm, wob_hbm,
            o_hbm,
            x_scr, wq_scr, wo_scr, kv_scr, acc_ref, ost_ref,
            q_scr, ota_scr, otb_scr, X0, X1, X2, X3, zs, kv_sem, w_sem, x_sem, o_sem):
    sp = (X0, X1, X2, X3)
    x_hbm = (xa_hbm, xb_hbm)
    kv_hbm = (ka_hbm, va_hbm, kb_hbm, vb_hbm)
    wq_hbm = (wqa_hbm, wqb_hbm)
    wo_hbm = (woa_hbm, wob_hbm)
    f2u = lambda a: pltpu.bitcast(a, U32)
    u2f = lambda a: pltpu.bitcast(a, F32)
    u2b = lambda a: pltpu.bitcast(a, BF16)

    def x_copy(br, b):
        return pltpu.make_async_copy(x_hbm[br].at[b], x_scr.at[br, b], x_sem.at[br, b])

    def wq_copy(br, p):
        s = p & 3
        return pltpu.make_async_copy(wq_hbm[br].at[:, pl.ds(pl.multiple_of(p * PW, 128), PW)],
                                     wq_scr.at[br, s], w_sem.at[br, s])

    def wo_copy(br, p):
        s = p & 3
        return pltpu.make_async_copy(wo_hbm[br].at[pl.ds(pl.multiple_of(p * PW, 128), PW), :],
                                     wo_scr.at[br, s], w_sem.at[2 + br, s])

    def kv_starts(j):
        s = j & (R - 1)
        for a in range(4):
            pltpu.make_async_copy(kv_hbm[a].at[j & 7, pl.ds((j >> 3) * 2, 2)],
                                  kv_scr.at[s, a], kv_sem.at[s]).start()

    def kv_wait(j):
        s = j & (R - 1)
        pltpu.make_async_copy(kv_scr.at[s], kv_scr.at[s], kv_sem.at[s]).wait()

    def o_copy(b):
        return pltpu.make_async_copy(ost_ref.at[b], o_hbm.at[b], o_sem.at[b])

    def out_start(b):
        ost_ref[b] = acc_ref[b].astype(BF16)
        o_copy(b).start()

    def stages():
        zz = [zs[n] for n in range(NZ)]
        z, z2 = zz[0], zz[1]
        XW = [sp[u].at[z] for u in range(4)]
        XR = [sp[u].at[z2] for u in range(4)]
        ot_scr = [ota_scr.at[z], otb_scr.at[z]]

        def Q(br, p, b):
            q = jnp.dot(x_scr[br, b], wq_scr[br, p & 3], preferred_element_type=F32)
            q = (q * (SCALE * LOG2E)).astype(BF16)
            for hh in range(2):
                q_scr[br * 2 + hh, z, :, 0:DH] = f2u(q[:, hh * DH:(hh + 1) * DH])

        def S(br, hh, slot):
            u = br * 2 + hh
            qh = u2b(q_scr[u, z, :, 0:DH])
            XW[u][0:SQ, :] = f2u(jnp.dot(qh, kv_scr[slot, 2 * br, hh], preferred_element_type=F32))

        def P1(br, hh):
            u = br * 2 + hh
            for r in range(0, SQ, RC):
                s = u2f(XW[u][r:r + RC, :])
                m = jnp.max(s, axis=-1, keepdims=True)
                XW[u][MO + r:MO + r + RC, 0:128] = f2u(jnp.broadcast_to(m, (RC, 128)))

        def P2(br, hh):
            u = br * 2 + hh
            items = [(r, c) for r in range(0, SQ, RC) for c in range(0, SK, CW)]

            def ld(it):
                r, c = it
                s = u2f(XR[u][r:r + RC, c:c + CW])
                m = u2f(XR[u][MO + r:MO + r + RC, 0:128]) if c == 0 else None
                return s, m
            pend = [ld(items[0])]
            mb = l = None
            for n, (r, c) in enumerate(items):
                if n + 1 < len(items):
                    pend.append(ld(items[n + 1]))
                s, m = pend.pop(0)
                if c == 0:
                    mb, l = m, None
                ps = [jnp.exp2(s[:, cc * 128:(cc + 1) * 128] - mb) for cc in range(CW // 128)]
                for pc in ps:
                    l = pc if l is None else l + pc
                p = jnp.concatenate(ps, axis=1).astype(BF16)
                XW[u][PO + r // 2:PO + (r + RC) // 2, c:c + CW] = f2u(p)
                if c + CW == SK:
                    XW[u][MO + r:MO + r + RC, 128:256] = f2u(l)

        def O(br, hh, slot):
            u = br * 2 + hh
            lp = u2f(XR[u][MO:MO + SP, 128:256])
            rt = 1.0 / jnp.sum(lp.T, axis=0, keepdims=True)
            for n in range(2):
                a0, a1 = n * 128, (n + 1) * 128
                v = kv_scr[slot + zz[n], 2 * br + 1, hh]
                p = u2b(XR[u][PO + a0 // 2:PO + a1 // 2, :])
                ot = lax.dot_general(v, p, NT, preferred_element_type=F32)
                ot_scr[br][hh * 96:(hh + 1) * 96, a0:a1] = f2u((ot * rt[:, a0:a1]).astype(BF16))

        def Y(br, p, b):
            o = u2b(ot_scr[br][...]).T[:SQ]
            y = jnp.dot(o, wo_scr[br, p & 3], preferred_element_type=F32)
            acc_ref[b, :, br * D:(br + 1) * D] += y
        return Q, S, P1, P2, O, Y

    for br in range(2):
        x_copy(br, 0).start()
        wq_copy(br, 0).start()
    kv_starts(0)
    for br in range(2):
        wo_copy(br, 0).start()
        x_copy(br, 1).start()
    for br in range(2):
        wq_copy(br, 1).start()
        for bb in range(2, B):
            x_copy(br, bb).start()
    for n in range(NZ):
        zs[n] = 0
    acc_ref[...] = jnp.zeros(acc_ref.shape, F32)
    otb_scr[...] = jnp.zeros(otb_scr.shape, U32)
    for u in range(4):
        sp[u][0, PO + SQ // 2:MO, :] = jnp.zeros((MO - PO - SQ // 2, SK), U32)
        sp[u][0, MO + SQ:MO + SP, 128:256] = f2u(jnp.ones((SP - SQ, 128), F32))
    Q, S, P1, P2, O, Y = stages()
    for br in range(2):
        x_copy(br, 0).wait()
        wq_copy(br, 0).wait()
        Q(br, 0, 0)

    def body(j, _):
        p = j >> 3
        b = j & 7

        @pl.when((b == 0) | (p == 0) | (j >= NJ - 6))
        def _():
            @pl.when(b == 0)
            def _():
                for br in range(2):
                    wo_copy(br, p).wait()

                @pl.when(p + 1 < NPAIR)
                def _():
                    for br in range(2):
                        wq_copy(br, p + 1).wait()
                        wo_copy(br, p + 1).start()

                @pl.when(p + 2 < NPAIR)
                def _():
                    for br in range(2):
                        wq_copy(br, p + 2).start()

            @pl.when((p == 0) & (b + 1 < B))
            def _():
                for br in range(2):
                    x_copy(br, b + 1).wait()

            @pl.when(j >= NJ - 6)
            def _():
                out_start((j - 2) & 7)

        slot = j & (R - 1)
        kv_wait(j)

        @pl.when(j + R - 1 < NJ)
        def _():
            kv_starts(j + R - 1)

        Q, S, P1, P2, O, Y = stages()
        j1 = jnp.minimum(j + 1, NJ - 1)
        p1, b1 = j1 >> 3, j1 & 7
        jm = jnp.maximum(j - 1, 0)
        pm, bm = jm >> 3, jm & 7

        S(0, 0, slot)
        S(0, 1, slot)
        P1(0, 0)
        P2(0, 0)
        Y(1, pm, bm)
        P1(0, 1)
        O(0, 0, slot)
        P2(0, 1)
        S(1, 0, slot)
        O(0, 1, slot)
        S(1, 1, slot)
        P1(1, 0)
        P2(1, 0)
        Q(0, p1, b1)
        O(1, 0, slot)
        P1(1, 1)
        P2(1, 1)
        Y(0, p, b)
        Q(1, p1, b1)
        O(1, 1, slot)

    lax.fori_loop(0, NJ, body, None)

    out_start(B - 2)
    Y(1, NPAIR - 1, B - 1)
    out_start(B - 1)
    for bb in range(B):
        o_copy(bb).wait()


@jax.jit
def pallas_concat_heads__gqa_block_cached__gqa_block_cached__near_ridge_kernel(
    A_x: jax.Array,
    A_k_cache: jax.Array,
    A_v_cache: jax.Array,
    A_wq: jax.Array,
    A_wo: jax.Array,
    B_x: jax.Array,
    B_k_cache: jax.Array,
    B_v_cache: jax.Array,
    B_wq: jax.Array,
    B_wo: jax.Array,
):
    t = lambda a: jnp.swapaxes(a, 2, 3)
    V = pltpu.VMEM
    any_spec = pl.BlockSpec(memory_space=pl.ANY)
    return pl.pallas_call(
        _kernel,
        in_specs=[any_spec] * 10,
        out_specs=any_spec,
        out_shape=jax.ShapeDtypeStruct((B, SQ, 2 * D), BF16),
        scratch_shapes=[V((2, B, SQ, D), BF16), V((2, 4, D, PW), BF16), V((2, 4, PW, D), BF16),
                        V((R, 4, 2, DH, SK), BF16),
                        V((B, SQ, 2 * D), F32), V((B, SQ, 2 * D), BF16),
                        V((4, 1, SQ // 2, 256), U32)]
        + [V((1, DH, SP), U32)] * 2
        + [V((1, XR_, SK), U32)] * 4 + [pltpu.SMEM((8,), jnp.int32)]
        + [pltpu.SemaphoreType.DMA((R,)), pltpu.SemaphoreType.DMA((4, 4)),
           pltpu.SemaphoreType.DMA((2, B)), pltpu.SemaphoreType.DMA((B,))],
        compiler_params=pltpu.CompilerParams(
            vmem_limit_bytes=100 * 1024 * 1024, disable_bounds_checks=True),
    )(A_x, B_x, t(A_k_cache), t(A_v_cache), t(B_k_cache), t(B_v_cache), A_wq, A_wo, B_wq, B_wo)
```

```python
import jax
import jax.numpy as jnp
import numpy as np
from jax import lax
import jax.experimental.pallas as pl
import jax.experimental.pallas.tpu as pltpu


B, SQ, D = 8, 240, 640
H, SK, DH = 32, 1024, 192
PW = 2 * DH
NPAIR = H // 2
NJ = NPAIR * B
SPS = 2
NSTEP = NJ // SPS
R = 2
SCALE = DH ** -0.5
LOG2E = float(np.log2(np.e))
F32 = jnp.float32
BF16 = jnp.bfloat16
U32 = jnp.uint32
NT = (((1,), (1,)), ((), ()))

RC = 16
CW = 512
SP = 256
PO = SQ
MO = PO + SP // 2
XROWS = MO + SP
NZ = 3

ORDER0 = 'S00 S01 Y1 S10 S11 O00 O01 O10 Q0 Y0 O11 Q1'
ORDER1 = 'S00 S01 Y1 S10 O00 O01 S11 O10 Q1 Q0 Y0 O11'


def _kernel(xa_hbm, xb_hbm, ka_hbm, va_hbm, kb_hbm, vb_hbm, wqa_hbm, woa_hbm, wqb_hbm, wob_hbm,
            o_hbm,
            x_scr, wq_scr, wo_scr, kv_scr, acc_ref, ost_ref,
            q_scr, ota_scr, otb_scr, X0, X1, X2, X3, zs, kv_sem, i_sem, w_sem, x_sem, o_sem):
    sp = (X0, X1, X2, X3)
    x_hbm = (xa_hbm, xb_hbm)
    kv_hbm = (ka_hbm, va_hbm, kb_hbm, vb_hbm)
    wq_hbm = (wqa_hbm, wqb_hbm)
    wo_hbm = (woa_hbm, wob_hbm)
    f2u = lambda a: pltpu.bitcast(a, U32)
    u2f = lambda a: pltpu.bitcast(a, F32)
    u2b = lambda a: pltpu.bitcast(a, BF16)

    def x_copy(br, b):
        return pltpu.make_async_copy(x_hbm[br].at[b], x_scr.at[br, b], x_sem.at[br, b])

    def wq_copy(br, p):
        s = p & 3
        return pltpu.make_async_copy(wq_hbm[br].at[:, pl.ds(pl.multiple_of(p * PW, 128), PW)],
                                     wq_scr.at[br, s], w_sem.at[br, s])

    def wo_copy(br, p):
        s = p & 3
        return pltpu.make_async_copy(wo_hbm[br].at[pl.ds(pl.multiple_of(p * PW, 128), PW), :],
                                     wo_scr.at[br, s], w_sem.at[2 + br, s])

    def kv_starts(st):
        j = st * SPS
        s = st & (R - 1)
        for a in range(4):
            pltpu.make_async_copy(kv_hbm[a].at[pl.ds(j & 7, SPS), pl.ds((j >> 3) * 2, 2)],
                                  kv_scr.at[s, a], kv_sem.at[s]).start()

    def kv_wait(st):
        s = st & (R - 1)
        pltpu.make_async_copy(kv_scr.at[s], kv_scr.at[s], kv_sem.at[s]).wait()

    def kv0_copy(t, a):
        return pltpu.make_async_copy(kv_hbm[a].at[t, pl.ds(0, 2)], kv_scr.at[0, a, t], i_sem.at[t, a])

    def o_copy(b):
        return pltpu.make_async_copy(ost_ref.at[b], o_hbm.at[b], o_sem.at[b])

    def out_start(b):
        ost_ref[b] = acc_ref[b].astype(BF16)
        o_copy(b).start()

    def stages():
        zz = [zs[n] for n in range(NZ)]
        z, z2 = zz[0], zz[1]
        XW = [sp[u].at[z] for u in range(4)]
        XR = [sp[u].at[z2] for u in range(4)]
        ot_scr = [ota_scr.at[z], otb_scr.at[z]]

        def Q(br, p, b):
            q = jnp.dot(x_scr[br, b], wq_scr[br, p & 3], preferred_element_type=F32)
            q = (q * (SCALE * LOG2E)).astype(BF16)
            for hh in range(2):
                q_scr[br * 2 + hh, z, :, 0:DH] = f2u(q[:, hh * DH:(hh + 1) * DH])

        def S(br, hh, slot, t):
            u = br * 2 + hh
            qh = u2b(q_scr[u, z, :, 0:DH])
            XW[u][0:SQ, :] = f2u(jnp.dot(qh, kv_scr[slot, 2 * br, t, hh], preferred_element_type=F32))

        def P1(br, hh):
            u = br * 2 + hh
            for r in range(0, SQ, RC):
                s = u2f(XW[u][r:r + RC, :])
                m = jnp.max(s, axis=-1, keepdims=True)
                XW[u][MO + r:MO + r + RC, 0:128] = f2u(jnp.broadcast_to(m, (RC, 128)))

        def P2(br, hh):
            u = br * 2 + hh
            items = [(r, c) for r in range(0, SQ, RC) for c in range(0, SK, CW)]

            def ld(it):
                r, c = it
                s = u2f(XR[u][r:r + RC, c:c + CW])
                m = u2f(XR[u][MO + r:MO + r + RC, 0:128]) if c == 0 else None
                return s, m
            pend = [ld(items[0])]
            mb = l = None
            for n, (r, c) in enumerate(items):
                if n + 1 < len(items):
                    pend.append(ld(items[n + 1]))
                s, m = pend.pop(0)
                if c == 0:
                    mb, l = m, None
                ps = [jnp.exp2(s[:, cc * 128:(cc + 1) * 128] - mb) for cc in range(CW // 128)]
                for pc in ps:
                    l = pc if l is None else l + pc
                p = jnp.concatenate(ps, axis=1).astype(BF16)
                XW[u][PO + r // 2:PO + (r + RC) // 2, c:c + CW] = f2u(p)
                if c + CW == SK:
                    XW[u][MO + r:MO + r + RC, 128:256] = f2u(l)

        def O(br, hh, slot, t):
            u = br * 2 + hh
            lp = u2f(XR[u][MO:MO + SP, 128:256])
            rt = 1.0 / jnp.sum(lp.T, axis=0, keepdims=True)
            for n in range(2):
                a0, a1 = n * 128, (n + 1) * 128
                v = kv_scr[slot + zz[n], 2 * br + 1, t, hh]
                p = u2b(XR[u][PO + a0 // 2:PO + a1 // 2, :])
                ot = lax.dot_general(v, p, NT, preferred_element_type=F32)
                ot_scr[br][hh * (DH // 2):(hh + 1) * (DH // 2), a0:a1] = f2u((ot * rt[:, a0:a1]).astype(BF16))

        def Y(br, p, b):
            o = u2b(ot_scr[br][...]).T[:SQ]
            y = jnp.dot(o, wo_scr[br, p & 3], preferred_element_type=F32)
            acc_ref[b, :, br * D:(br + 1) * D] += y
        return Q, S, P1, P2, O, Y

    def iteration(st, j, slot, t, order, pre=None, first=False):
        Q, S, P1, P2, O, Y = st
        p, b = j >> 3, j & 7
        j1 = min(j + 1, NJ - 1) if isinstance(j, int) else jnp.minimum(j + 1, NJ - 1)
        jm = j - 1
        for op in order.split():
            if pre and op in pre:
                pre[op]()
            k, br = op[0], int(op[1])
            if k == 'S':
                S(br, int(op[2]), slot, t)
                P1(br, int(op[2]))
                P2(br, int(op[2]))
            elif k == 'O':
                O(br, int(op[2]), slot, t)
            elif k == 'Q':
                Q(br, j1 >> 3, j1 & 7)
            elif br == 0:
                Y(0, p, b)
            elif not first:
                Y(1, jm >> 3, jm & 7)

    def manage(i):
        j0 = i * SPS
        p = j0 >> 3
        b0 = j0 & 7

        @pl.when((b0 == 0) | (b0 == B - SPS) | (p == 0) | (j0 >= NJ - B + SPS))
        def _():
            @pl.when(b0 == 0)
            def _():
                for br in range(2):
                    wo_copy(br, p).wait()

                @pl.when(p + 1 < NPAIR)
                def _():
                    for br in range(2):
                        wq_copy(br, p + 1).start()
                        wo_copy(br, p + 1).start()

            @pl.when((b0 == B - SPS) & (p + 1 < NPAIR))
            def _():
                for br in range(2):
                    wq_copy(br, p + 1).wait()

            @pl.when(p == 0)
            def _():
                for d in (1, 2):
                    @pl.when(b0 + d < B)
                    def _():
                        for br in range(2):
                            x_copy(br, b0 + d).wait()
                for d in (3, 4):
                    @pl.when(b0 + d < B)
                    def _():
                        for br in range(2):
                            x_copy(br, b0 + d).start()

            @pl.when(j0 - 2 >= NJ - B)
            def _():
                for t in range(SPS):
                    jp = j0 - 2 - t

                    @pl.when(jp >= NJ - B)
                    def _():
                        out_start(jp & 7)
        kv_wait(i)

    for br in range(2):
        x_copy(br, 0).start()
        wq_copy(br, 0).start()
    kv0_copy(0, 0).start()
    kv0_copy(0, 2).start()
    for n in range(NZ):
        zs[n] = 0
    acc_ref[...] = jnp.zeros(acc_ref.shape, F32)
    for u in range(4):
        sp[u][0, PO + SQ // 2:MO, :] = jnp.zeros((MO - PO - SQ // 2, SK), U32)
        sp[u][0, MO + SQ:MO + SP, 128:256] = f2u(jnp.ones((SP - SQ, 128), F32))
    st = stages()
    x_copy(0, 0).wait()
    wq_copy(0, 0).wait()
    kv0_copy(0, 1).start()
    st[0](0, 0, 0)
    x_copy(1, 0).wait()
    wq_copy(1, 0).wait()
    kv0_copy(0, 3).start()
    st[0](1, 0, 0)

    def need_ka():
        kv0_copy(0, 0).wait()
        for br in range(2):
            x_copy(br, 1).start()

    def need_kb():
        kv0_copy(0, 2).wait()
        for br in range(2):
            wo_copy(br, 0).start()

    def need_va():
        kv0_copy(0, 1).wait()
        kv0_copy(1, 0).start()

    def need_vb():
        kv0_copy(0, 3).wait()
        kv0_copy(1, 1).start()
        kv0_copy(1, 2).start()

    def need_x1():
        for br in range(2):
            x_copy(br, 1).wait()
        kv0_copy(1, 3).start()

    def need_wo():
        for br in range(2):
            wo_copy(br, 0).wait()
            x_copy(br, 2).start()

    pre = {'S00': need_ka, 'S10': need_kb, 'O00': need_va, 'O10': need_vb, 'Q0': need_x1, 'Y0': need_wo}
    iteration(st, 0, 0, 0, ORDER0, pre=pre, first=True)
    for a in range(4):
        kv0_copy(1, a).wait()
    for br in range(2):
        x_copy(br, 2).wait()
    kv_starts(1)
    for br in range(2):
        x_copy(br, 3).start()
        x_copy(br, 4).start()
    iteration(st, 1, 0, 1, ORDER1)
    manage(jnp.int32(1))
    kv_starts(2)
    for br in range(2):
        wq_copy(br, 1).start()
        wo_copy(br, 1).start()

    def body(i, _):
        slot = i & (R - 1)
        st_i = stages()
        iteration(st_i, SPS * i, slot, 0, ORDER0)
        iteration(st_i, SPS * i + 1, slot, 1, ORDER1)

        @pl.when(i + R < NSTEP)
        def _():
            kv_starts(i + R)

        @pl.when(i + 1 < NSTEP)
        def _():
            manage(i + 1)

    lax.fori_loop(1, NSTEP, body, None)

    out_start(B - 3)
    out_start(B - 2)
    st[5](1, NPAIR - 1, B - 1)
    out_start(B - 1)
    for bb in range(B):
        o_copy(bb).wait()


@jax.jit
def pallas_concat_heads__gqa_block_cached__gqa_block_cached__near_ridge_kernel(
    A_x: jax.Array,
    A_k_cache: jax.Array,
    A_v_cache: jax.Array,
    A_wq: jax.Array,
    A_wo: jax.Array,
    B_x: jax.Array,
    B_k_cache: jax.Array,
    B_v_cache: jax.Array,
    B_wq: jax.Array,
    B_wo: jax.Array,
):
    t = lambda a: jnp.swapaxes(a, 2, 3)
    V = pltpu.VMEM
    any_spec = pl.BlockSpec(memory_space=pl.ANY)
    return pl.pallas_call(
        _kernel,
        in_specs=[any_spec] * 10,
        out_specs=any_spec,
        out_shape=jax.ShapeDtypeStruct((B, SQ, 2 * D), BF16),
        scratch_shapes=[V((2, B, SQ, D), BF16), V((2, 4, D, PW), BF16), V((2, 4, PW, D), BF16),
                        V((R, 4, SPS, 2, DH, SK), BF16),
                        V((B, SQ, 2 * D), F32), V((B, SQ, 2 * D), BF16),
                        V((4, 1, SQ // 2, 256), U32)]
        + [V((1, DH, SP), U32)] * 2
        + [V((1, XROWS, SK), U32)] * 4 + [pltpu.SMEM((8,), jnp.int32)]
        + [pltpu.SemaphoreType.DMA((R,)), pltpu.SemaphoreType.DMA((2, 4)), pltpu.SemaphoreType.DMA((4, 4)),
           pltpu.SemaphoreType.DMA((2, B)), pltpu.SemaphoreType.DMA((B,))],
        compiler_params=pltpu.CompilerParams(
            vmem_limit_bytes=100 * 1024 * 1024, disable_bounds_checks=True),
    )(A_x, B_x, t(A_k_cache), t(A_v_cache), t(B_k_cache), t(B_v_cache), A_wq, A_wo, B_wq, B_wo)
```

```python
import jax
import jax.numpy as jnp
import numpy as np
from jax import lax
import jax.experimental.pallas as pl
import jax.experimental.pallas.tpu as pltpu


B, SQ, D = 8, 240, 640
H, SK, DH = 32, 1024, 192
PW = 2 * DH
NPAIR = H // 2
NJ = NPAIR * B
SPS = 2
NSTEP = NJ // SPS
R = 2
SCALE = DH ** -0.5
LOG2E = float(np.log2(np.e))
F32 = jnp.float32
BF16 = jnp.bfloat16
U32 = jnp.uint32
NT = (((1,), (1,)), ((), ()))

RC = 16
CW = 512
SP = 256
PO = SQ
MO = PO + SP // 2
XROWS = MO + SP
NZ = 3

ORDER0 = 'S00 S01 Y1 S10 S11 O00 O01 O10 Q0 Y0 O11 Q1'
ORDER1 = 'S00 S01 Y1 S10 O00 O01 S11 O10 Q1 Q0 Y0 O11'
ORDERW = 'S00 S01 Y1 O00 S10 O01 S11 Q0 O10 Y0 Q1 O11'
NWARM = 4


def _kernel(xa_hbm, xb_hbm, ka_hbm, va_hbm, kb_hbm, vb_hbm, wqa_hbm, woa_hbm, wqb_hbm, wob_hbm,
            o_hbm,
            x_scr, wq_scr, wo_scr, kv_scr, acc_ref, ost_ref,
            q_scr, ota_scr, otb_scr, X0, X1, X2, X3, zs, kv_sem, i_sem, w_sem, x_sem, o_sem):
    sp = (X0, X1, X2, X3)
    x_hbm = (xa_hbm, xb_hbm)
    kv_hbm = (ka_hbm, va_hbm, kb_hbm, vb_hbm)
    wq_hbm = (wqa_hbm, wqb_hbm)
    wo_hbm = (woa_hbm, wob_hbm)
    f2u = lambda a: pltpu.bitcast(a, U32)
    u2f = lambda a: pltpu.bitcast(a, F32)
    u2b = lambda a: pltpu.bitcast(a, BF16)

    def x_copy(br, b):
        return pltpu.make_async_copy(x_hbm[br].at[b], x_scr.at[br, b], x_sem.at[br, b])

    def wq_copy(br, p):
        s = p & 3
        return pltpu.make_async_copy(wq_hbm[br].at[:, pl.ds(pl.multiple_of(p * PW, 128), PW)],
                                     wq_scr.at[br, s], w_sem.at[br, s])

    def wo_copy(br, p):
        s = p & 3
        return pltpu.make_async_copy(wo_hbm[br].at[pl.ds(pl.multiple_of(p * PW, 128), PW), :],
                                     wo_scr.at[br, s], w_sem.at[2 + br, s])

    def kv_starts(st):
        j = st * SPS
        s = st & (R - 1)
        for a in range(4):
            pltpu.make_async_copy(kv_hbm[a].at[pl.ds(j & 7, SPS), pl.ds((j >> 3) * 2, 2)],
                                  kv_scr.at[s, a], kv_sem.at[s]).start()

    def kv_wait(st):
        s = st & (R - 1)
        pltpu.make_async_copy(kv_scr.at[s], kv_scr.at[s], kv_sem.at[s]).wait()

    def kv0_copy(j, a):
        return pltpu.make_async_copy(kv_hbm[a].at[j, pl.ds(0, 2)], kv_scr.at[j >> 1, a, j & 1], i_sem.at[j, a])

    def o_copy(b):
        return pltpu.make_async_copy(ost_ref.at[b], o_hbm.at[b], o_sem.at[b])

    def out_start(b):
        ost_ref[b] = acc_ref[b].astype(BF16)
        o_copy(b).start()

    def stages():
        zz = [zs[n] for n in range(NZ)]
        z, z2 = zz[0], zz[1]
        XW = [sp[u].at[z] for u in range(4)]
        XR = [sp[u].at[z2] for u in range(4)]
        ot_scr = [ota_scr.at[z], otb_scr.at[z]]

        def Q(br, p, b):
            q = jnp.dot(x_scr[br, b], wq_scr[br, p & 3], preferred_element_type=F32)
            q = (q * (SCALE * LOG2E)).astype(BF16)
            for hh in range(2):
                q_scr[br * 2 + hh, z, :, 0:DH] = f2u(q[:, hh * DH:(hh + 1) * DH])

        def S(br, hh, slot, t):
            u = br * 2 + hh
            qh = u2b(q_scr[u, z, :, 0:DH])
            XW[u][0:SQ, :] = f2u(jnp.dot(qh, kv_scr[slot, 2 * br, t, hh], preferred_element_type=F32))

        def P1(br, hh):
            u = br * 2 + hh
            for r in range(0, SQ, RC):
                s = u2f(XW[u][r:r + RC, :])
                m = jnp.max(s, axis=-1, keepdims=True)
                XW[u][MO + r:MO + r + RC, 0:128] = f2u(jnp.broadcast_to(m, (RC, 128)))

        def P2(br, hh):
            u = br * 2 + hh
            items = [(r, c) for r in range(0, SQ, RC) for c in range(0, SK, CW)]

            def ld(it):
                r, c = it
                s = u2f(XR[u][r:r + RC, c:c + CW])
                m = u2f(XR[u][MO + r:MO + r + RC, 0:128]) if c == 0 else None
                return s, m
            pend = [ld(items[0])]
            mb = l = None
            for n, (r, c) in enumerate(items):
                if n + 1 < len(items):
                    pend.append(ld(items[n + 1]))
                s, m = pend.pop(0)
                if c == 0:
                    mb, l = m, None
                ps = [jnp.exp2(s[:, cc * 128:(cc + 1) * 128] - mb) for cc in range(CW // 128)]
                for pc in ps:
                    l = pc if l is None else l + pc
                p = jnp.concatenate(ps, axis=1).astype(BF16)
                XW[u][PO + r // 2:PO + (r + RC) // 2, c:c + CW] = f2u(p)
                if c + CW == SK:
                    XW[u][MO + r:MO + r + RC, 128:256] = f2u(l)

        def O(br, hh, slot, t):
            u = br * 2 + hh
            lp = u2f(XR[u][MO:MO + SP, 128:256])
            rt = 1.0 / jnp.sum(lp.T, axis=0, keepdims=True)
            for n in range(2):
                a0, a1 = n * 128, (n + 1) * 128
                v = kv_scr[slot + zz[n], 2 * br + 1, t, hh]
                p = u2b(XR[u][PO + a0 // 2:PO + a1 // 2, :])
                ot = lax.dot_general(v, p, NT, preferred_element_type=F32)
                ot_scr[br][hh * (DH // 2):(hh + 1) * (DH // 2), a0:a1] = f2u((ot * rt[:, a0:a1]).astype(BF16))

        def Y(br, p, b):
            o = u2b(ot_scr[br][...]).T[:SQ]
            y = jnp.dot(o, wo_scr[br, p & 3], preferred_element_type=F32)
            acc_ref[b, :, br * D:(br + 1) * D] += y
        return Q, S, P1, P2, O, Y

    def iteration(st, j, slot, t, order, pre=None, first=False):
        Q, S, P1, P2, O, Y = st
        p, b = j >> 3, j & 7
        j1 = min(j + 1, NJ - 1) if isinstance(j, int) else jnp.minimum(j + 1, NJ - 1)
        jm = j - 1
        for op in order.split():
            if pre and op in pre:
                pre[op]()
            k, br = op[0], int(op[1])
            if k == 'S':
                S(br, int(op[2]), slot, t)
                P1(br, int(op[2]))
                P2(br, int(op[2]))
            elif k == 'O':
                O(br, int(op[2]), slot, t)
            elif k == 'Q':
                Q(br, j1 >> 3, j1 & 7)
            elif br == 0:
                Y(0, p, b)
            elif not first:
                Y(1, jm >> 3, jm & 7)

    def manage(i):
        j0 = i * SPS
        p = j0 >> 3
        b0 = j0 & 7

        @pl.when((b0 == 0) | (b0 == B - SPS) | (p == 0) | (j0 >= NJ - B + SPS))
        def _():
            @pl.when(b0 == 0)
            def _():
                for br in range(2):
                    wo_copy(br, p).wait()

                @pl.when(p + 1 < NPAIR)
                def _():
                    for br in range(2):
                        wq_copy(br, p + 1).start()
                        wo_copy(br, p + 1).start()

            @pl.when((b0 == B - SPS) & (p + 1 < NPAIR))
            def _():
                for br in range(2):
                    wq_copy(br, p + 1).wait()

            @pl.when(p == 0)
            def _():
                for d in (1, 2):
                    @pl.when(b0 + d < B)
                    def _():
                        for br in range(2):
                            x_copy(br, b0 + d).wait()
                for d in (3, 4):
                    @pl.when(b0 + d < B)
                    def _():
                        for br in range(2):
                            x_copy(br, b0 + d).start()

            @pl.when(j0 - 2 >= NJ - B)
            def _():
                for t in range(SPS):
                    jp = j0 - 2 - t

                    @pl.when(jp >= NJ - B)
                    def _():
                        out_start(jp & 7)
        kv_wait(i)

    KA, VA, KB, VB = range(4)

    def start(copies):
        return lambda: [c().start() for c in copies]

    def wait(copies):
        return lambda: [c().wait() for c in copies]

    def both(*fs):
        return lambda: [f() for f in fs]

    kv = lambda j, *arrs: [(lambda a=a: kv0_copy(j, a)) for a in arrs]
    xs = lambda *bs: [(lambda br=br, b=b: x_copy(br, b)) for b in bs for br in range(2)]
    wo0 = [(lambda br=br: wo_copy(br, 0)) for br in range(2)]
    it_data = lambda j: kv(j, KA, VA, KB, VB) + xs(j + 1)

    for br in range(2):
        x_copy(br, 0).start()
        wq_copy(br, 0).start()
    start(kv(0, KA, KB))()
    for n in range(NZ):
        zs[n] = 0
    acc_ref[...] = jnp.zeros(acc_ref.shape, F32)
    for u in range(4):
        sp[u][0, PO + SQ // 2:MO, :] = jnp.zeros((MO - PO - SQ // 2, SK), U32)
        sp[u][0, MO + SQ:MO + SP, 128:256] = f2u(jnp.ones((SP - SQ, 128), F32))
    st = stages()
    for br in range(2):
        x_copy(br, 0).wait()
        wq_copy(br, 0).wait()
        kv0_copy(0, VA if br == 0 else VB).start()
        st[0](br, 0, 0)

    iteration(st, 0, 0, 0, ORDERW, first=True, pre={
        'S00': both(wait(kv(0, KA)), start(xs(1))),
        'O00': both(wait(kv(0, VA, KB)), start(wo0 + kv(1, KA))),
        'Q0': both(wait(xs(1) + kv(0, VB)), start(kv(1, VA, KB, VB))),
        'Y0': both(wait(wo0), start(xs(2)))})
    iteration(st, 1, 0, 1, ORDERW, pre={
        'S00': both(wait(it_data(1)), start(it_data(2))),
        'Q0': start(it_data(3))})
    iteration(st, 2, 1, 0, ORDERW, pre={
        'S00': wait(it_data(2)),
        'O01': both(lambda: kv_starts(2), start(xs(5, 6)))})
    iteration(st, 3, 1, 1, ORDERW, pre={'S00': wait(it_data(3))})
    manage(jnp.int32(2))
    kv_starts(3)
    for br in range(2):
        wq_copy(br, 1).start()
        wo_copy(br, 1).start()

    def body(i, _):
        slot = i & (R - 1)
        st_i = stages()
        iteration(st_i, SPS * i, slot, 0, ORDER0)
        iteration(st_i, SPS * i + 1, slot, 1, ORDER1)

        @pl.when(i + R < NSTEP)
        def _():
            kv_starts(i + R)

        @pl.when(i + 1 < NSTEP)
        def _():
            manage(i + 1)

    lax.fori_loop(NWARM // SPS, NSTEP, body, None)

    out_start(B - 3)
    out_start(B - 2)
    st[5](1, NPAIR - 1, B - 1)
    out_start(B - 1)
    for bb in range(B):
        o_copy(bb).wait()


@jax.jit
def pallas_concat_heads__gqa_block_cached__gqa_block_cached__near_ridge_kernel(
    A_x: jax.Array,
    A_k_cache: jax.Array,
    A_v_cache: jax.Array,
    A_wq: jax.Array,
    A_wo: jax.Array,
    B_x: jax.Array,
    B_k_cache: jax.Array,
    B_v_cache: jax.Array,
    B_wq: jax.Array,
    B_wo: jax.Array,
):
    t = lambda a: jnp.swapaxes(a, 2, 3)
    V = pltpu.VMEM
    any_spec = pl.BlockSpec(memory_space=pl.ANY)
    return pl.pallas_call(
        _kernel,
        in_specs=[any_spec] * 10,
        out_specs=any_spec,
        out_shape=jax.ShapeDtypeStruct((B, SQ, 2 * D), BF16),
        scratch_shapes=[V((2, B, SQ, D), BF16), V((2, 4, D, PW), BF16), V((2, 4, PW, D), BF16),
                        V((R, 4, SPS, 2, DH, SK), BF16),
                        V((B, SQ, 2 * D), F32), V((B, SQ, 2 * D), BF16),
                        V((4, 1, SQ // 2, 256), U32)]
        + [V((1, DH, SP), U32)] * 2
        + [V((1, XROWS, SK), U32)] * 4 + [pltpu.SMEM((8,), jnp.int32)]
        + [pltpu.SemaphoreType.DMA((R,)), pltpu.SemaphoreType.DMA((NWARM, 4)), pltpu.SemaphoreType.DMA((4, 4)),
           pltpu.SemaphoreType.DMA((2, B)), pltpu.SemaphoreType.DMA((B,))],
        compiler_params=pltpu.CompilerParams(
            vmem_limit_bytes=100 * 1024 * 1024, disable_bounds_checks=True),
    )(A_x, B_x, t(A_k_cache), t(A_v_cache), t(B_k_cache), t(B_v_cache), A_wq, A_wo, B_wq, B_wo)
```
